```python
import os as _os
_os.environ.setdefault("JAX_PLATFORMS", "cpu")
import jax
import jax.numpy as jnp

def _softmax(x, axis=-1):
    return jax.nn.softmax(x, axis=axis)
def _gelu(x):
    return jax.nn.gelu(x, approximate=True)
def _silu(x):
    return jax.nn.silu(x)
def _sigmoid(x):
    return jax.nn.sigmoid(x)
def _layernorm(x, axis=-1, eps=1e-5):
    m = jnp.mean(x, axis=axis, keepdims=True)
    v = jnp.var(x, axis=axis, keepdims=True)
    return (x - m) / jnp.sqrt(v + eps)
def _scatter_add(tgt, idx, src, axis=0):
    return tgt.at[idx].add(src)
def _segment_sum(src, seg, n):
    return jax.ops.segment_sum(src, seg, n)
class _Rng:
    def __init__(self, key):
        self._k = key
    def _next(self):
        self._k, sub = jax.random.split(self._k)
        return sub
    def normal(self, shape):
        return jax.random.normal(self._next(), shape, dtype=jnp.bfloat16)
    def randint(self, lo, hi, shape):
        return jax.random.randint(self._next(), shape, lo, hi, dtype=jnp.int32)
    def uniform(self, shape, lo=0.0, hi=1.0):
        return jax.random.uniform(self._next(), shape, jnp.bfloat16, lo, hi)
    def permutation(self, n):
        return jax.random.permutation(self._next(), n)


kernel_name = 'gated_mix__sliding_local_dilated__moe_arch_mod__prompt'

def setup_inputs():
    _rng = _Rng(jax.random.key(int.from_bytes(__import__("os").urandom(4), "little")))
    _w = (lambda a: (lambda t: t.astype(jnp.bfloat16) if jnp.issubdtype(t.dtype, jnp.floating) else t)(jnp.asarray(a)))
    def _A_setup():
        B, S, D = 1, 2048, 640
        return {
            "x": _w((lambda *s: _rng.normal(s) * 0.05)(B, S, D)),
            "wqkv": _w((lambda *s: _rng.normal(s) * 0.8)(D, 3 * D)),
            "wo": _w((lambda *s: _rng.normal(s) * 0.05)(D, D)),
        }
    _A_in = _A_setup()

    def _B_setup():
        B, S, D, F, C = 1, 2048, 640, 1728, 1
        return {
            "x": _w((lambda *s: _rng.normal(s) * 0.05)(B, S, D)),
            "w_r": _w((lambda *s: _rng.normal(s) * 1.6)(D)),
            "w_gate": _w((lambda *s: _rng.normal(s) * 0.4)(D, F)),
            "w_up": _w((lambda *s: _rng.normal(s) * 0.4)(D, F)),
            "w_down": _w((lambda *s: _rng.normal(s) * 0.4)(F, D)),
        }
    _B_in = _B_setup()

    return {
        "A_x": _A_in["x"],
        "A_wqkv": _A_in["wqkv"],
        "A_wo": _A_in["wo"],
        "B_x": _B_in["x"],
        "B_w_r": _B_in["w_r"],
        "B_w_gate": _B_in["w_gate"],
        "B_w_up": _B_in["w_up"],
        "B_w_down": _B_in["w_down"],
        "gate_w": _w((lambda *s: _rng.normal(s) * 0.05)(640) * 16.0),
    }

def reference(A_x, A_wqkv, A_wo, B_x, B_w_r, B_w_gate, B_w_up, B_w_down, gate_w):
    def _A_ref(x, wqkv, wo):
        B, S, D = x.shape
        H = 32; Dh = D // H
        W, dil = 8, 2
        qkv = (lambda x, *d: x.transpose(*d))((x @ wqkv).reshape(B, S, 3, H, Dh), 2, 0, 3, 1, 4)
        q, k, v = qkv[0], qkv[1], qkv[2]
        scale = Dh ** -0.5
        pos = jnp.arange(S)
        off = jnp.arange(W) * dil
        idx = pos[:, None] - off[None, :]
        mask = idx >= 0
        idx_c = jnp.where(mask, idx, 0).reshape(-1)
        kg = k[:, :, idx_c, :].reshape(B, H, S, W, Dh)
        vg = v[:, :, idx_c, :].reshape(B, H, S, W, Dh)
        logits = jnp.einsum("bhsd,bhswd->bhsw", q, kg) * scale
        logits = jnp.where(mask[None, None, :, :], logits, -1e9)
        attn = _softmax(logits, axis=-1)
        o = jnp.einsum("bhsw,bhswd->bhsd", attn, vg)
        return (lambda x, *d: x.transpose(*d))(o, 0, 2, 1, 3).reshape(B, S, D) @ wo

    def _B_ref(x, w_r, w_gate, w_up, w_down):
        B, S, D = x.shape
        C = 1
        r = x @ w_r
        idx = jnp.argsort(-r, axis=-1)[:, :C]
        idx_e = jnp.repeat(idx.reshape(B, C, 1), D, axis=2)
        x_sel = jnp.take_along_axis(x, idx_e, axis=1)
        g = _silu(x_sel @ w_gate)
        u = x_sel @ w_up
        y = (g * u) @ w_down
        r_sel = _sigmoid(jnp.take_along_axis(r, idx, axis=1))
        y = y * r_sel.reshape(B, C, 1)
        b_off = (jnp.arange(B) * S).reshape(B, 1)
        flat_idx = (idx + b_off).reshape(B * C)
        zero = (x * 0.0).reshape(B * S, D)
        upd = _scatter_add(zero, flat_idx, y.reshape(B * C, D), axis=0)
        return x + upd.reshape(B, S, D)

    x = A_x
    g = _sigmoid((x * gate_w).sum(-1, keepdims=True))
    a = _A_ref(x, A_wqkv, A_wo)
    b = _B_ref(x, B_w_r, B_w_gate, B_w_up, B_w_down)
    return g * a + (1 - g) * b
```

```python
import functools
import math

import jax
import jax.numpy as jnp
import jax.experimental.pallas as pl
import jax.experimental.pallas.tpu as pltpu

S, D, F = 2048, 640, 1728
H, DH, WIN, DIL = 32, 20, 8, 2
NT = D // 128
HALO = 16
LOG2E = math.log2(math.e)
QSCALE = (DH ** -0.5) * LOG2E
NEG = -1e9 * LOG2E
F32 = jnp.float32
BF16 = jnp.bfloat16
U32 = jnp.uint32
I32 = jnp.int32


def _sigmoid(z):
    return 0.5 * jnp.tanh(0.5 * z) + 0.5


def _rows8(v):
    return [v[8 * j:8 * j + 8] for j in range(v.shape[0] // 8)]


def _kernel(x_hbm, wqkv_hbm, wo_hbm, wr_hbm, wg_hbm, wu_hbm, wd_hbm, gw_hbm,
            out_hbm,
            x_v, wqkv_v, wo_v, wr_v, gw_v, wg_v, wu_v, wd_v,
            wqp_v, wkvp_v, wof_v, wop_v, q_s, k_s, v_s, o_s, g_s, xg_s, out_v,
            sem_in, sem_out, *, cfg):
    xt = cfg["x_tiles"]
    pm = cfg["piece"]
    ot = cfg["out_tiles"]
    npc = S // pm

    def cp(src, dst, i):
        return pltpu.make_async_copy(src, dst, sem_in.at[i])

    n = 0
    c_wq = cp(wqkv_hbm.at[:, 0:D], wqkv_v.at[:, 0:D], n); n += 1
    c_x = []
    for i in range(len(xt) - 1):
        c_x.append(cp(x_hbm.at[0, xt[i]:xt[i + 1], :], x_v.at[xt[i]:xt[i + 1], :], n)); n += 1
    c_wk = cp(wqkv_hbm.at[:, D:2 * D], wqkv_v.at[:, D:2 * D], n); n += 1
    c_wv = cp(wqkv_hbm.at[:, 2 * D:3 * D], wqkv_v.at[:, 2 * D:3 * D], n); n += 1
    c_wo = cp(wo_hbm, wo_v, n); n += 1
    c_wr = cp(wr_hbm, wr_v, n); n += 1
    c_gw = cp(gw_hbm, gw_v, n); n += 1
    c_wg = cp(wg_hbm, wg_v, n); n += 1
    c_wu = cp(wu_hbm, wu_v, n); n += 1
    c_wd = cp(wd_hbm, wd_v, n); n += 1

    c_wr.start()
    c_gw.start()
    c_wq.start()
    for c in c_x:
        c.start()
    c_wk.start()
    c_wv.start()
    c_wo.start()
    c_wg.start()
    c_wu.start()
    c_wd.start()

    for t in range(NT):
        k_s[t, 0:HALO, :] = jnp.zeros((HALO, 128), F32)
        v_s[t, 0:HALO, :] = jnp.zeros((HALO, 128), F32)

    c_wr.wait()
    c_gw.wait()
    wr = wr_v[...].reshape(1, D).astype(F32)
    gw = gw_v[...].reshape(1, D).astype(F32)
    vi = pltpu.bitcast(jnp.broadcast_to(wr[:, 0:128], (8, 128)), I32)
    vz = jnp.maximum(jnp.minimum(vi, 0), 0)
    mfalse = vz != 0
    zi = jnp.max(vz)

    def gated_weights(w_ref, col, gates):
        gates = [pltpu.bitcast(g, U32) for g in gates]
        ng_ = len(gates)
        assert ng_ <= D // 16, ng_
        parts = [jnp.where(mfalse, g, w_ref[8 * j:8 * j + 8, col:col + 128]) for j, g in enumerate(gates)]
        if ng_ < D // 16:
            parts.append(w_ref[8 * ng_:D // 2, col:col + 128])
        w = parts[0] if len(parts) == 1 else jnp.concatenate(parts, axis=0)
        return pltpu.bitcast(w, BF16)

    def perm_task(part, r0, prb):
        lane = jax.lax.broadcasted_iota(I32, (prb // 2, 128), 1)
        lm5 = lane % 5
        src = [pltpu.bitcast(
            wqkv_v[r0:r0 + prb, part * D + t * 128: part * D + (t + 1) * 128], U32)
            for t in range(NT)]
        gates = []
        for t in range(NT):
            bl = src[0]
            for s in range(1, NT):
                bl = jnp.where(lm5 == (t - 3 * s) % 5, src[s], bl)
            pat = ((lane & 31) * DH + 5 * (lane >> 5) + t) & 127
            g = jnp.take_along_axis(bl, pat, axis=1, mode="promise_in_bounds")
            if part == 0:
                wqp_v[r0 // 2:(r0 + prb) // 2, t * 128:(t + 1) * 128] = g
            else:
                c0 = (part - 1) * D + t * 128
                wkvp_v[r0 // 2:(r0 + prb) // 2, c0:c0 + 128] = g
            gates += _rows8(g)
        return gates

    def wo_task(j, t):
        if t == 0:
            wof_v[j] = wo_v[:, j * 128:(j + 1) * 128].astype(F32)
        gates = []
        for c in range(4):
            rows = wof_v[j, pl.ds(5 * c + t, H, stride=DH), :]
            r0 = t * 128 + c * H
            pk = pltpu.bitcast(rows.astype(BF16), U32)
            wop_v[r0 // 2:(r0 + H) // 2, j * 128:(j + 1) * 128] = pk
            gates += _rows8(pk)
        return gates

    sub = jax.lax.broadcasted_iota(I32, (8, 128), 0)
    st = dict(best_v=jnp.full((8, 128), -jnp.inf, F32), best_i=jnp.zeros((8, 128), I32))
    rvals = {}

    def rg_task(r0):
        xf16 = x_v[r0:r0 + 16, :].astype(F32)
        gates = []
        for hh in range(2):
            xf = xf16[hh * 8:(hh + 1) * 8]
            xs = [xf[:, t * 128:(t + 1) * 128] for t in range(NT)]
            pr = xs[0] * wr[:, 0:128]
            pg = xs[0] * gw[:, 0:128]
            for t in range(1, NT):
                pr = pr + xs[t] * wr[:, t * 128:(t + 1) * 128]
                pg = pg + xs[t] * gw[:, t * 128:(t + 1) * 128]
            rr = r0 + hh * 8
            rvals[rr] = jnp.broadcast_to(jnp.sum(pr, axis=1, keepdims=True), (8, 128))
            gates.append(rvals[rr])
            g = jnp.broadcast_to(_sigmoid(jnp.sum(pg, axis=1, keepdims=True)), (8, 128))
            g_s[rr:rr + 8, :] = g
            omg = 1.0 - g
            for t in range(NT):
                xg = omg * xs[t]
                xg_s[t, rr:rr + 8, :] = xg
                gates.append(xg)
        return gates

    def argmax_task(a, b):
        for rr in range(a, b, 8):
            rv = rvals.pop(rr).astype(BF16).astype(F32)
            upd = rv > st["best_v"]
            st["best_v"] = jnp.where(upd, rv, st["best_v"])
            st["best_i"] = jnp.where(upd, sub + rr, st["best_i"])
        return [st["best_v"], st["best_i"]]

    def sel_task():
        best_v, best_i = st["best_v"], st["best_i"]
        top_v = jnp.max(best_v, axis=0, keepdims=True)
        cand = jnp.where(best_v == top_v, best_i, S)
        top_i = jnp.min(cand, axis=0, keepdims=True)
        idx = jnp.clip(jnp.min(top_i), 0, S - 1)
        base = pl.multiple_of((idx >> 4) << 4, 16)
        xblk = x_v[pl.ds(base, 16), :].astype(F32)
        rsel = jax.lax.broadcasted_iota(I32, (16, D), 0) == (idx - base)
        x_sel = jnp.sum(jnp.where(rsel, xblk, 0.0), axis=0, keepdims=True)
        st.update(top_v=top_v, top_i=top_i, base=base, x_sel=x_sel)
        return []

    accs = [jnp.zeros((8, 128), F32) for _ in range(NT)]
    hvals = {}

    def gu_task(k0):
        x_sel = st["x_sel"]
        gt = jnp.sum(wg_v[k0:k0 + 16, :].astype(F32) * x_sel, axis=1, keepdims=True)
        ut = jnp.sum(wu_v[k0:k0 + 16, :].astype(F32) * x_sel, axis=1, keepdims=True)
        hvals[k0] = jnp.broadcast_to(gt * _sigmoid(gt) * ut, (16, 128))
        return _rows8(hvals[k0])

    def dn_task(k0, k1):
        for k in range(k0, k1, 16):
            hc = hvals.pop(k)
            for t in range(NT):
                p = wd_v[k:k + 16, t * 128:(t + 1) * 128].astype(F32) * hc
                accs[t] = accs[t] + (p[0:8] + p[8:16])
        return list(accs)

    def ffn_fin():
        gsel = _sigmoid(jnp.sum(st["x_sel"] * gw, axis=1, keepdims=True))
        sc = _sigmoid(st["top_v"]) * (1.0 - gsel)
        st["y"] = [jnp.sum(accs[t], axis=0, keepdims=True) * sc for t in range(NT)]
        return []

    def attn_chunk(r0):
        qs = [q_s[t, r0:r0 + 8, :] for t in range(NT)]
        ps = []
        for w in range(WIN):
            off = HALO + r0 - DIL * w
            acc = qs[0] * k_s[0, off:off + 8, :]
            for t in range(1, NT):
                acc = acc + qs[t] * k_s[t, off:off + 8, :]
            ps.append(acc)
        ps = [p + pltpu.roll(p, 64, 1) for p in ps]
        logits = [p + pltpu.roll(p, 32, 1) for p in ps]
        for w in range(WIN):
            if r0 < DIL * w:
                logits[w] = jnp.where(sub + r0 >= DIL * w, logits[w], NEG)
        m = logits[0]
        for w in range(1, WIN):
            m = jnp.maximum(m, logits[w])
        es = [jnp.exp2(l - m) for l in logits]
        den = es[0]
        for w in range(1, WIN):
            den = den + es[w]
        rc = pl.reciprocal(den, approx=True)
        inv = rc * (2.0 - den * rc)
        outs = []
        for t in range(NT):
            off = HALO + r0
            acc = es[0] * v_s[t, off:off + 8, :]
            for w in range(1, WIN):
                off = HALO + r0 - DIL * w
                acc = acc + es[w] * v_s[t, off:off + 8, :]
            outs.append(acc * inv)
        return outs

    def attn_task(r0):
        lo = attn_chunk(r0)
        hi = attn_chunk(r0 + 8)
        gates = []
        for t in range(NT):
            o16 = pltpu.bitcast(jnp.concatenate([lo[t], hi[t]], axis=0).astype(BF16), U32)
            o_s[r0 // 2:r0 // 2 + 8, t * 128:(t + 1) * 128] = o16
            gates.append(o16)
        return gates

    outs_dma = []

    def send_task(j):
        a, b = ot[j], ot[j + 1]
        y = st["y"]
        pb = pl.multiple_of(jnp.clip(st["base"], a, b - 16), 16)
        hit = (jax.lax.broadcasted_iota(I32, (16, 128), 0) + pb) == st["top_i"]
        for t in range(NT):
            cur = out_v[pl.ds(pb, 16), t * 128:(t + 1) * 128].astype(F32)
            out_v[pl.ds(pb, 16), t * 128:(t + 1) * 128] = (cur + jnp.where(hit, y[t], 0.0)).astype(BF16)
        c = pltpu.make_async_copy(out_v.at[a:b, :], out_hbm.at[0, a:b, :], sem_out.at[j])
        c.start()
        outs_dma.append(c)
        return []

    def out_fence():
        r = pl.multiple_of(S + zi * 16, 16)
        out_v[pl.ds(r, 16), 0:128] = jnp.zeros((16, 128), BF16)
        return [out_v[pl.ds(r, 16), 0:128]]

    olag = cfg["out_lag"]
    slots = [("q", p, t) for p in range(npc) for t in range(NT)]
    n1 = len(slots)
    for i in range(npc + olag):
        if i < npc:
            slots += [("kv", i, t) for t in range(2 * NT)]
        if i >= olag:
            slots += [("wo", i - olag, t) for t in range(NT)]
    ns = len(slots)
    pos = {s: n_ for n_, s in enumerate(slots)}
    tasks = [[] for _ in range(ns + 1)]
    waits = {}

    def spread(fns, s0, s1):
        for n_, fn in enumerate(fns):
            tasks[s0 + (s1 - s0) * (n_ + 1) // len(fns)].append(fn)

    blk = cfg["blackout"]
    fw1, fw2, f1 = n1 + cfg["gu_wait"], n1 + cfg["dn_wait"], n1 + cfg["ffn_end"]
    starts = [pos[("q", xt[i] // pm, 0)] for i in range(len(xt) - 1)] + [fw1]
    for i in range(len(xt) - 1):
        s0 = starts[i]
        s1 = starts[i + 1] if i < len(xt) - 2 else n1 + cfg["rg_tail"]
        waits[s0] = [c_x[i]]
        spread([functools.partial(rg_task, r0) for r0 in range(xt[i], xt[i + 1], 16)], s0 + blk - 1, s1)
        if i < len(xt) - 2:
            na = cfg["argmax_n"]
            cuts = [xt[i] + (xt[i + 1] - xt[i]) // 8 * j // na * 8 for j in range(na + 1)]
            spread([functools.partial(argmax_task, cuts[j], cuts[j + 1]) for j in range(na)],
                   starts[i + 1] + 1, starts[i + 1] + 1 + 2 * na)
    waits[s0] += [c_wk, c_wv, c_wo]
    prb = cfg["perm_rb"]
    spread([functools.partial(perm_task, p, r0, prb) for p in (1, 2) for r0 in range(0, D, prb)],
           s0 + blk - 1, n1 - 1)
    spread([functools.partial(wo_task, j, t) for j in range(NT) for t in range(NT)], n1, n1 + cfg["wo_span"])
    waits[fw1] = [c_wg, c_wu]
    waits[fw2] = [c_wd]
    tasks[fw1 + 1] += [functools.partial(argmax_task, xt[-2], xt[-1]), sel_task]
    spread([functools.partial(gu_task, k0) for k0 in range(0, F, 16)], fw1 + cfg["gu_off"], fw2)
    dg = cfg["dn_group"] * 16
    spread([functools.partial(dn_task, k0, min(k0 + dg, F)) for k0 in range(0, F, dg)], fw2 + 1, f1)
    tasks[f1 + 1].append(ffn_fin)
    aoff = cfg["attn_off"]
    a0 = pos[("kv", 0, 2 * NT - 1)] + 1 + aoff
    a1 = pos[("wo", npc - 1, 0)]
    allowed = [s for s in range(a0, a1 + 1) if not any(w < s < w + blk for w in (fw1, fw2))]
    npair = S // 16
    prev = 0
    for j in range(npair):
        p = j * 16 // pm
        s = allowed[(len(allowed) - 1) * j // (npair - 1)]
        lo_s = pos[("kv", p, 2 * NT - 1)] + 1 + aoff + (j % (pm // 16)) * cfg["attn_min_gap"]
        s = min(max(s, lo_s, prev), pos[("wo", p, 0)])
        while s not in allowed:
            s += 1
        prev = s
        tasks[s].append(functools.partial(attn_task, j * 16))
    for p in range(npc):
        s = min(pos[("wo", p, NT - 1)] + 1 + cfg["ofence_off"], ns)
        for j in range(len(ot) - 1):
            if ot[j + 1] == (p + 1) * pm:
                sj = max(s, f1 + 3)
                tasks[sj].append(functools.partial(send_task, j))
                if sj != s and sj < ns:
                    tasks[sj].append(out_fence)
        if s < ns:
            tasks[s].append(out_fence)

    c_wq.wait()
    for r0 in range(0, D, cfg["perm_rb0"]):
        perm_task(0, r0, cfg["perm_rb0"])

    carry = []
    for s in range(ns + 1):
        gates = carry
        for fn in tasks[s]:
            gates += fn()
        if s in waits:
            for c in waits[s]:
                c.wait()
            gates = []
        if s == ns:
            break
        gates, carry = gates[:D // 16], gates[D // 16:]
        kind, p, t = slots[s]
        a, b = p * pm, (p + 1) * pm
        if t == 0 or s in waits:
            lhs = pltpu.bitcast(o_s[a // 2:b // 2, :], BF16) if kind == "wo" else x_v[a:b, :]
        if kind == "q":
            q = jnp.dot(lhs, gated_weights(wqp_v, t * 128, gates), preferred_element_type=F32)
            q_s[t, a:b, :] = q * QSCALE
        elif kind == "kv":
            r = jnp.dot(lhs, gated_weights(wkvp_v, t * 128, gates), preferred_element_type=F32)
            if t < NT:
                k_s[t, HALO + a:HALO + b, :] = r
            else:
                v_s[t - NT, HALO + a:HALO + b, :] = r
        else:
            att = jnp.dot(lhs, gated_weights(wop_v, t * 128, gates),
                          preferred_element_type=F32)
            out_v[a:b, t * 128:(t + 1) * 128] = (g_s[a:b, :] * att + xg_s[t, a:b, :]).astype(BF16)
    assert len(outs_dma) == len(ot) - 1
    for c in outs_dma:
        c.wait()


_CFG = dict(
    x_tiles=(0, 384, 1408, 2048),
    piece=128,
    out_tiles=(0, 1152, 1408, 1664, 1792, 1920, 2048),
    perm_rb0=320, perm_rb=32, blackout=3, rg_tail=8, argmax_n=4, wo_span=30,
    out_lag=3, attn_off=3, attn_min_gap=1, ofence_off=5,
    gu_wait=34, gu_off=5, dn_wait=100, ffn_end=165, dn_group=2,
)


def _build(cfg):
    hbm = pl.BlockSpec(memory_space=pltpu.HBM)
    n_in = 9 + len(cfg["x_tiles"]) - 1
    n_out = len(cfg["out_tiles"]) - 1
    return pl.pallas_call(
        functools.partial(_kernel, cfg=cfg),
        out_shape=jax.ShapeDtypeStruct((1, S, D), BF16),
        in_specs=[hbm] * 8,
        out_specs=hbm,
        scratch_shapes=[
            pltpu.VMEM((S, D), BF16),
            pltpu.VMEM((D, 3 * D), BF16),
            pltpu.VMEM((D, D), BF16),
            pltpu.VMEM((D,), BF16),
            pltpu.VMEM((D,), BF16),
            pltpu.VMEM((F, D), BF16),
            pltpu.VMEM((F, D), BF16),
            pltpu.VMEM((F, D), BF16),
            pltpu.VMEM((D // 2, D), U32),
            pltpu.VMEM((D // 2, 2 * D), U32),
            pltpu.VMEM((NT, D, 128), F32),
            pltpu.VMEM((D // 2, D), U32),
            pltpu.VMEM((NT, S, 128), F32),
            pltpu.VMEM((NT, S + HALO, 128), F32),
            pltpu.VMEM((NT, S + HALO, 128), F32),
            pltpu.VMEM((S // 2, D), U32),
            pltpu.VMEM((S, 128), F32),
            pltpu.VMEM((NT, S, 128), F32),
            pltpu.VMEM((S + 16, D), BF16),
            pltpu.SemaphoreType.DMA((n_in,)),
            pltpu.SemaphoreType.DMA((n_out,)),
        ],
        compiler_params=pltpu.CompilerParams(vmem_limit_bytes=100 * 1024 * 1024),
        name="gated_mix_kernel",
    )


@jax.jit
def pallas_gated_mix__sliding_local_dilated__moe_arch_mod__prompt_kernel(
    A_x, A_wqkv, A_wo, B_x, B_w_r, B_w_gate, B_w_up, B_w_down, gate_w):
    del B_x
    return _build(_CFG)(A_x, A_wqkv, A_wo, B_w_r, B_w_gate.T, B_w_up.T, B_w_down, gate_w)
```

```python
import functools
import math

import jax
import jax.numpy as jnp
import jax.experimental.pallas as pl
import jax.experimental.pallas.tpu as pltpu

S, D, F = 2048, 640, 1728
H, DH, WIN, DIL = 32, 20, 8, 2
NT = D // 128
HALO = 16
LOG2E = math.log2(math.e)
QSCALE = (DH ** -0.5) * LOG2E
NEG = -1e9 * LOG2E
F32 = jnp.float32
BF16 = jnp.bfloat16
U32 = jnp.uint32
I32 = jnp.int32


def _sigmoid(z):
    return 0.5 * jnp.tanh(0.5 * z) + 0.5


def _rows8(v):
    return [v[8 * j:8 * j + 8] for j in range(v.shape[0] // 8)]


def _kernel(x_hbm, wqkv_hbm, wo_hbm, wr_hbm, wg_hbm, wu_hbm, wd_hbm, gw_hbm,
            out_hbm,
            x_v, wqkv_v, wo_v, wr_v, gw_v, wg_v, wu_v, wd_v,
            wqp_v, wkvp_v, wof_v, wop_v, q_s, k_s, v_s, o_s, g_s, xg_s, out_v, xu_s,
            sem_in, sem_out, *, cfg):
    xt = cfg["x_tiles"]
    pm = cfg["piece"]
    ot = cfg["out_tiles"]
    npc = S // pm

    def cp(src, dst, i):
        return pltpu.make_async_copy(src, dst, sem_in.at[i])

    nx = len(xt) - 1
    ka = cfg["ka"]
    c_wr = cp(wr_hbm, wr_v, 0)
    c_gw = cp(gw_hbm, gw_v, 0)
    c_wqa = cp(wqkv_hbm.at[0:ka, 0:D], wqkv_v.at[0:ka, 0:D], 1)
    c_x = [cp(x_hbm.at[0, xt[i]:xt[i + 1], :], x_v.at[xt[i]:xt[i + 1], :], 2 + i) for i in range(nx)]
    c_wqb = cp(wqkv_hbm.at[ka:D, 0:D], wqkv_v.at[ka:D, 0:D], 3)
    c_wk = cp(wqkv_hbm.at[:, D:2 * D], wqkv_v.at[:, D:2 * D], 1 + nx)
    c_wv = cp(wqkv_hbm.at[:, 2 * D:3 * D], wqkv_v.at[:, 2 * D:3 * D], 1 + nx)
    c_wo = cp(wo_hbm, wo_v, 1 + nx)
    c_wg = cp(wg_hbm, wg_v, 2 + nx)
    c_wu = cp(wu_hbm, wu_v, 2 + nx)
    c_wd = cp(wd_hbm, wd_v, 3 + nx)

    c_wr.start()
    c_gw.start()
    c_wqa.start()
    c_x[0].start()
    c_wqb.start()
    for c in c_x[1:]:
        c.start()
    c_wk.start()
    c_wv.start()
    c_wo.start()
    c_wg.start()
    c_wu.start()
    c_wd.start()

    for t in range(NT):
        k_s[t, 0:HALO, :] = jnp.zeros((HALO, 128), F32)
        v_s[t, 0:HALO, :] = jnp.zeros((HALO, 128), F32)

    c_wr.wait()
    c_gw.wait()
    wr = wr_v[...].reshape(1, D).astype(F32)
    gw = gw_v[...].reshape(1, D).astype(F32)
    vi = pltpu.bitcast(jnp.broadcast_to(wr[:, 0:128], (8, 128)), I32)
    vz = jnp.maximum(jnp.minimum(vi, 0), 0)
    mfalse = vz != 0
    zi = jnp.max(vz)

    def gated_weights(w_ref, col, gates, k0=0, k1=D):
        gates = [pltpu.bitcast(g, U32) for g in gates]
        lo, hi = k0 // 2, k1 // 2
        parts = [jnp.where(mfalse, g, w_ref[lo + 8 * j:lo + 8 * j + 8, col:col + 128]) for j, g in enumerate(gates)]
        if lo + 8 * len(gates) < hi:
            parts.append(w_ref[lo + 8 * len(gates):hi, col:col + 128])
        w = parts[0] if len(parts) == 1 else jnp.concatenate(parts, axis=0)
        return pltpu.bitcast(w, BF16)

    def perm_task(part, r0, prb):
        lane = jax.lax.broadcasted_iota(I32, (prb // 2, 128), 1)
        lm5 = lane % 5
        src = [pltpu.bitcast(
            wqkv_v[r0:r0 + prb, part * D + t * 128: part * D + (t + 1) * 128], U32)
            for t in range(NT)]
        gates = []
        for t in range(NT):
            bl = src[0]
            for s in range(1, NT):
                bl = jnp.where(lm5 == (t - 3 * s) % 5, src[s], bl)
            pat = ((lane & 31) * DH + 5 * (lane >> 5) + t) & 127
            g = jnp.take_along_axis(bl, pat, axis=1, mode="promise_in_bounds")
            if part == 0:
                wqp_v[r0 // 2:(r0 + prb) // 2, t * 128:(t + 1) * 128] = g
            else:
                c0 = (part - 1) * D + t * 128
                wkvp_v[r0 // 2:(r0 + prb) // 2, c0:c0 + 128] = g
            gates += _rows8(g)
        return gates

    def wo_task(j, t):
        if t == 0:
            z = st["late_z"] if cfg["wo_late"] else 0
            for r0 in range(0, D, 128):
                rr = pl.multiple_of(r0 + z * 16, 16) if cfg["wo_late"] else r0
                wof_v[j, r0:r0 + 128, :] = wo_v[pl.ds(rr, 128), j * 128:(j + 1) * 128].astype(F32)
        gates = []
        for c in range(4):
            d = 5 * c + t
            ev = wof_v[j, pl.ds(d, H // 2, stride=2 * DH), :]
            od = wof_v[j, pl.ds(d + DH, H // 2, stride=2 * DH), :]
            pk = pltpu.pack_elementwise([ev, od], packed_dtype=BF16)
            r0 = (t * 128 + c * H) // 2
            wop_v[r0:r0 + H // 2, j * 128:(j + 1) * 128] = pk
            gates += _rows8(pk)
        return gates

    sub = jax.lax.broadcasted_iota(I32, (8, 128), 0)
    st = dict(best_v=jnp.full((8, 128), -jnp.inf, F32), best_i=jnp.zeros((8, 128), I32))
    rvals = {}

    def rg_task(r0):
        xf16 = x_v[r0:r0 + 16, :].astype(F32)
        gates = []
        for hh in range(2):
            xf = xf16[hh * 8:(hh + 1) * 8]
            xs = [xf[:, t * 128:(t + 1) * 128] for t in range(NT)]
            pr = xs[0] * wr[:, 0:128]
            pg = xs[0] * gw[:, 0:128]
            for t in range(1, NT):
                pr = pr + xs[t] * wr[:, t * 128:(t + 1) * 128]
                pg = pg + xs[t] * gw[:, t * 128:(t + 1) * 128]
            rr = r0 + hh * 8
            rvals[rr] = jnp.broadcast_to(jnp.sum(pr, axis=1, keepdims=True), (8, 128))
            gates.append(rvals[rr])
            g = jnp.broadcast_to(_sigmoid(jnp.sum(pg, axis=1, keepdims=True)), (8, 128))
            g_s[rr:rr + 8, :] = g
            omg = 1.0 - g
            for t in range(NT):
                xg = omg * xs[t]
                xg_s[t, rr:rr + 8, :] = xg
                gates.append(xg)
        return gates

    def argmax_task(a, b):
        for rr in range(a, b, 8):
            rv = rvals.pop(rr).astype(BF16).astype(F32)
            upd = rv > st["best_v"]
            st["best_v"] = jnp.where(upd, rv, st["best_v"])
            st["best_i"] = jnp.where(upd, sub + rr, st["best_i"])
        return [st["best_v"], st["best_i"]]

    def sel_task():
        best_v, best_i = st["best_v"], st["best_i"]
        top_v = jnp.max(best_v, axis=0, keepdims=True)
        cand = jnp.where(best_v == top_v, best_i, S)
        top_i = jnp.min(cand, axis=0, keepdims=True)
        idx = jnp.clip(jnp.min(top_i), 0, S - 1)
        base = pl.multiple_of((idx >> 4) << 4, 16)
        xblk = x_v[pl.ds(base, 16), :].astype(F32)
        rsel = jax.lax.broadcasted_iota(I32, (16, D), 0) == (idx - base)
        x_sel = jnp.sum(jnp.where(rsel, xblk, 0.0), axis=0, keepdims=True)
        st.update(top_v=top_v, top_i=top_i, base=base, x_sel=x_sel)
        return []

    accs = [jnp.zeros((8, 128), F32) for _ in range(NT)]
    hvals = {}

    def gu_task(k0):
        x_sel = st["x_sel"]
        gt = jnp.sum(wg_v[k0:k0 + 16, :].astype(F32) * x_sel, axis=1, keepdims=True)
        ut = jnp.sum(wu_v[k0:k0 + 16, :].astype(F32) * x_sel, axis=1, keepdims=True)
        hvals[k0] = jnp.broadcast_to(gt * _sigmoid(gt) * ut, (16, 128))
        return _rows8(hvals[k0])

    def dn_task(k0, k1):
        for k in range(k0, k1, 16):
            hc = hvals.pop(k)
            for t in range(NT):
                p = wd_v[k:k + 16, t * 128:(t + 1) * 128].astype(F32) * hc
                accs[t] = accs[t] + (p[0:8] + p[8:16])
        return list(accs)

    def ffn_fin(done_rows):
        gsel = _sigmoid(jnp.sum(st["x_sel"] * gw, axis=1, keepdims=True))
        sc = _sigmoid(st["top_v"]) * (1.0 - gsel)
        y = [jnp.sum(accs[t], axis=0, keepdims=True) * sc for t in range(NT)]
        row16 = jax.lax.broadcasted_iota(I32, (16, 128), 0)
        base = st["base"]
        hit = (row16 + base) == st["top_i"]
        pb = pl.multiple_of(jnp.minimum(base, done_rows - 16), 16)
        hit2 = (row16 + pb) == st["top_i"]
        for t in range(NT):
            xg_s[t, pl.ds(base, 16), :] = xg_s[t, pl.ds(base, 16), :] + jnp.where(hit, y[t], 0.0)
            cur = out_v[pl.ds(pb, 16), t * 128:(t + 1) * 128].astype(F32)
            out_v[pl.ds(pb, 16), t * 128:(t + 1) * 128] = (cur + jnp.where(hit2, y[t], 0.0)).astype(BF16)
        return []

    def attn_chunk(r0, tok):
        def rows(ref, t, off):
            return ref[t, pl.ds(off, 8, stride=2), :]
        qs = [rows(q_s, t, r0) for t in range(NT)]
        if tok is not None:
            for t in range(cfg["tok_n"]):
                qs[t] = jnp.where(mfalse, tok, qs[t])
        ps = []
        for w in range(WIN):
            off = HALO + r0 - DIL * w
            acc = qs[0] * rows(k_s, 0, off)
            for t in range(1, NT):
                acc = acc + qs[t] * rows(k_s, t, off)
            ps.append(acc)
        ps = [p + pltpu.roll(p, 64, 1) for p in ps]
        logits = [p + pltpu.roll(p, 32, 1) for p in ps]
        for w in range(WIN):
            if r0 < DIL * w:
                logits[w] = jnp.where(2 * sub + r0 >= DIL * w, logits[w], NEG)
        m = logits[0]
        for w in range(1, WIN):
            m = jnp.maximum(m, logits[w])
        es = [jnp.exp2(l - m) for l in logits]
        den = es[0]
        for w in range(1, WIN):
            den = den + es[w]
        rc = pl.reciprocal(den, approx=True)
        inv = rc * (2.0 - den * rc)
        outs = []
        for t in range(NT):
            acc = es[0] * rows(v_s, t, HALO + r0)
            for w in range(1, WIN):
                acc = acc + es[w] * rows(v_s, t, HALO + r0 - DIL * w)
            outs.append(acc * inv)
        return outs

    tokens = {}

    def attn_task(r0, s):
        tok = tokens.get(s - cfg["tok_w"])
        ev = attn_chunk(r0, tok)
        od = attn_chunk(r0 + 1, tok)
        gates = []
        for t in range(NT):
            o16 = pltpu.pack_elementwise([ev[t], od[t]], packed_dtype=BF16)
            o_s[r0 // 2:r0 // 2 + 8, t * 128:(t + 1) * 128] = o16
            gates.append(o16)
        return gates

    outs_dma = []

    def send_task(j):
        a, b = ot[j], ot[j + 1]
        c = pltpu.make_async_copy(out_v.at[a:b, :], out_hbm.at[0, a:b, :], sem_out.at[0])
        c.start()
        outs_dma.append(c)
        return []

    def out_fence():
        r = pl.multiple_of(S + zi * 16, 16)
        out_v[pl.ds(r, 16), 0:128] = jnp.zeros((16, 128), BF16)
        return [out_v[pl.ds(r, 16), 0:128]]

    olag = cfg["out_lag"]
    slots = [("qa", a, a + pm, t) for a in range(0, xt[2], pm) for t in range(NT)]
    slots += [("qb", a, a + pm, t) for a in range(0, xt[2], pm) for t in range(NT)]
    slots += [("q", a, a + pm, t) for a in range(xt[2], S, pm) for t in range(NT)]
    n1 = len(slots)
    wo_cuts = lambda p: [p * pm + c for c in cfg["last_cuts"]] if p == npc - 1 else [p * pm, (p + 1) * pm]
    for i in range(npc + olag):
        if i < npc:
            slots += [("kv", i * pm, (i + 1) * pm, t) for t in range(2 * NT)]
        if i >= olag:
            cuts = wo_cuts(i - olag)
            for a, b in zip(cuts[:-1], cuts[1:]):
                slots += [("wo", a, b, t) for t in range(NT)]
    ns = len(slots)
    first = {}
    last = {}
    for n_, (kind, a, b, t) in enumerate(slots):
        for r in range(a, b, 16):
            first.setdefault((kind, r), n_)
            last[(kind, r)] = n_
    tasks = [[] for _ in range(ns + 1)]
    waits = {}

    def spread(fns, s0, s1):
        for n_, fn in enumerate(fns):
            tasks[s0 + (s1 - s0) * (n_ + 1) // len(fns)].append(fn)

    blk = cfg["blackout"]
    fw1, fw2, f1 = n1 + cfg["gu_wait"], n1 + cfg["dn_wait"], n1 + cfg["ffn_end"]
    starts = [first[("qa" if i < 2 else "q", xt[i])] for i in range(len(xt) - 1)] + [fw1]
    for i in range(len(xt) - 1):
        s0 = starts[i]
        s1 = starts[i + 1] if i < len(xt) - 2 else n1 + cfg["rg_tail"]
        waits[s0] = [c_x[i]]
        spread([functools.partial(rg_task, r0) for r0 in range(xt[i], xt[i + 1], 16)],
               s0 + blk - 1 if i < len(xt) - 2 else n1 + cfg["rg_head"], s1)
        if i < len(xt) - 2:
            na = cfg["argmax_n"]
            cuts = [xt[i] + (xt[i + 1] - xt[i]) // 8 * j // na * 8 for j in range(na + 1)]
            spread([functools.partial(argmax_task, cuts[j], cuts[j + 1]) for j in range(na)],
                   starts[i + 1] + 1, starts[i + 1] + 1 + 2 * na)
    waits[s0] += [c_wk, c_wv, c_wo]
    waits[starts[1]] += [c_wqb]
    spread([functools.partial(perm_task, 0, r0, 32) for r0 in range(ka, D, 32)],
           starts[1] + cfg["permb_off"], first[("qb", 0)] - 1)
    prb = cfg["perm_rb"]
    mid = (s0 + blk - 1 + n1 + 4) // 2
    spread([functools.partial(perm_task, 1, r0, prb) for r0 in range(0, D, prb)], s0 + blk - 1, mid)
    spread([functools.partial(perm_task, 2, r0, prb) for r0 in range(0, D, prb)], mid, n1 + 4)
    spread([functools.partial(wo_task, j, t) for j in range(NT) for t in range(NT)],
           n1 + cfg["wo_0"], n1 + cfg["wo_span"])
    waits[fw1] = [c_wg, c_wu]
    waits[fw2] = [c_wd]
    tasks[fw1 + cfg['sel_off']] += [functools.partial(argmax_task, xt[-2], xt[-1]), sel_task]
    spread([functools.partial(gu_task, k0) for k0 in range(0, F, 16)], fw1 + cfg["gu_off"], fw2)
    dg = cfg["dn_group"] * 16
    spread([functools.partial(dn_task, k0, min(k0 + dg, F)) for k0 in range(0, F, dg)], fw2 + 1, f1)
    fin = last[("wo", ot[1] - 16)] + 1
    assert fin > f1, (fin, f1)
    tasks[fin].append(functools.partial(ffn_fin, ot[1]))
    aoff = cfg["attn_off"]
    a0 = last[("kv", 0)] + 1 + aoff
    a1 = first[("wo", S - 16)]
    allowed = [s for s in range(a0, a1 + 1) if not any(w < s < w + cfg['attn_blk'] for w in (fw1, fw2))]
    npair = S // 16
    prev = 0
    for j in range(npair):
        s = allowed[(len(allowed) - 1) * j // (npair - 1)]
        lo_s = last[("kv", j * 16)] + 1 + aoff + (j % (pm // 16)) * cfg["attn_min_gap"]
        s = min(max(s, lo_s, prev), first[("wo", j * 16)])
        while s not in allowed:
            s += 1
        prev = s
        tasks[s].append(functools.partial(attn_task, j * 16, s))
    for n_, (kind, a, b, t) in enumerate(slots):
        if kind == "wo" and t == NT - 1:
            if b in ot:
                tasks[n_ + 1].append(functools.partial(send_task, ot.index(b) - 1))
            s = n_ + 1 + cfg["ofence_off"] * pm // (b - a)
            if s < ns:
                tasks[n_ + 1].append(("fence", s))

    c_wqa.wait()
    for r0 in range(0, ka, cfg["perm_rb0"]):
        perm_task(0, r0, cfg["perm_rb0"])

    carry = []
    later = {}
    xl = {}
    qpart = {}
    for s in range(ns + 1):
        gates = carry + later.pop(s, [])
        for fn in tasks[s]:
            if isinstance(fn, tuple):
                later.setdefault(fn[1], []).extend(out_fence())
            else:
                gates += fn()
        if s in waits:
            for c in waits[s]:
                c.wait()
            gates = []
        if s == ns:
            break
        kind, a, b, t = slots[s]
        cap = {"qa": ka, "qb": D - ka}.get(kind, D) // 16
        gates, carry = gates[:cap], gates[cap:]
        if kind in ("qa", "q") and t == 0:
            xl[a] = x_v[a:b, :]
            if cfg["reload"]:
                xu_s[a // 2:b // 2, :] = pltpu.bitcast(xl[a], U32)
        if kind == "qa":
            qpart[(a, t)] = jnp.dot(xl[a][:, 0:ka], gated_weights(wqp_v, t * 128, gates, 0, ka),
                                    preferred_element_type=F32)
        elif kind == "qb":
            q = jnp.dot(xl[a][:, ka:D], gated_weights(wqp_v, t * 128, gates, ka, D), preferred_element_type=F32)
            q_s[t, a:b, :] = (q + qpart.pop((a, t))) * QSCALE
        elif kind == "q":
            q = jnp.dot(xl[a], gated_weights(wqp_v, t * 128, gates), preferred_element_type=F32)
            q_s[t, a:b, :] = q * QSCALE
        elif kind == "kv":
            if cfg["reload"]:
                if s == n1:
                    xu_s[pl.ds(pl.multiple_of(S // 2 + zi * 8, 8), 8), 0:128] = jnp.zeros((8, 128), U32)
                xl[a] = pltpu.bitcast(xu_s[a // 2:b // 2, :], BF16)
            r = jnp.dot(xl[a], gated_weights(wkvp_v, t * 128, gates), preferred_element_type=F32)
            if cfg["wo_late"] and s < n1 + cfg["wo_span"] and (s - n1) % 5 == 0:
                ri = pltpu.bitcast(r[0:8], I32)
                st["late_z"] = jnp.max(jnp.maximum(jnp.minimum(ri, 0), 0))
            tokens[s] = r[0:8]
            if t < NT:
                k_s[t, HALO + a:HALO + b, :] = r
            else:
                v_s[t - NT, HALO + a:HALO + b, :] = r
        else:
            if cfg["reload"] > 1:
                if t == 0:
                    o_s[pl.ds(pl.multiple_of(S // 2 + zi * 8, 8), 8), 0:128] = jnp.zeros((8, 128), U32)
                ol = pltpu.bitcast(o_s[a // 2:b // 2, :], BF16)
            elif t == 0:
                ol = pltpu.bitcast(o_s[a // 2:b // 2, :], BF16)
            att = jnp.dot(ol, gated_weights(wop_v, t * 128, gates), preferred_element_type=F32)
            tokens[s] = att[0:8]
            out_v[a:b, t * 128:(t + 1) * 128] = (g_s[a:b, :] * att + xg_s[t, a:b, :]).astype(BF16)
    assert len(outs_dma) == len(ot) - 1
    for c in outs_dma:
        c.wait()


_CFG = dict(
    x_tiles=(0, 256, 512, 1536, 2048), ka=384, permb_off=3,
    piece=128,
    out_tiles=(0, 1152, 1408, 1664, 1792, 1920, 1984, 2048),
    last_cuts=(0, 64, 128),
    perm_rb0=384, perm_rb=32, blackout=3, rg_head=-6, rg_tail=16, wo_0=4, wo_late=0, sel_off=3, tok_w=1000, reload=0, tok_n=1, attn_blk=4, argmax_n=4, wo_span=30,
    out_lag=3, attn_off=3, attn_min_gap=1, ofence_off=4, reuse_x=1,
    gu_wait=36, gu_off=6, dn_wait=100, ffn_end=160, dn_group=2,
)


def _build(cfg):
    hbm = pl.BlockSpec(memory_space=pltpu.HBM)
    n_in = 4 + len(cfg["x_tiles"]) - 1
    n_out = 1
    return pl.pallas_call(
        functools.partial(_kernel, cfg=cfg),
        out_shape=jax.ShapeDtypeStruct((1, S, D), BF16),
        in_specs=[hbm] * 8,
        out_specs=hbm,
        scratch_shapes=[
            pltpu.VMEM((S, D), BF16),
            pltpu.VMEM((D, 3 * D), BF16),
            pltpu.VMEM((D, D), BF16),
            pltpu.VMEM((D,), BF16),
            pltpu.VMEM((D,), BF16),
            pltpu.VMEM((F, D), BF16),
            pltpu.VMEM((F, D), BF16),
            pltpu.VMEM((F, D), BF16),
            pltpu.VMEM((D // 2, D), U32),
            pltpu.VMEM((D // 2, 2 * D), U32),
            pltpu.VMEM((NT, D + 40, 128), F32),
            pltpu.VMEM((D // 2, D), U32),
            pltpu.VMEM((NT, S + 8, 128), F32),
            pltpu.VMEM((NT, S + HALO + 8, 128), F32),
            pltpu.VMEM((NT, S + HALO + 8, 128), F32),
            pltpu.VMEM((S // 2 + 8, D), U32),
            pltpu.VMEM((S, 128), F32),
            pltpu.VMEM((NT, S, 128), F32),
            pltpu.VMEM((S + 16, D), BF16),
            pltpu.VMEM((S // 2 + 8, D), U32),
            pltpu.SemaphoreType.DMA((n_in,)),
            pltpu.SemaphoreType.DMA((n_out,)),
        ],
        compiler_params=pltpu.CompilerParams(vmem_limit_bytes=100 * 1024 * 1024),
        name="gated_mix_kernel",
    )


@jax.jit
def pallas_gated_mix__sliding_local_dilated__moe_arch_mod__prompt_kernel(
    A_x, A_wqkv, A_wo, B_x, B_w_r, B_w_gate, B_w_up, B_w_down, gate_w):
    del B_x
    return _build(_CFG)(A_x, A_wqkv, A_wo, B_w_r, B_w_gate.T, B_w_up.T, B_w_down, gate_w)
```

```python
import bisect
import functools
import math

import jax
import jax.numpy as jnp
import jax.experimental.pallas as pl
import jax.experimental.pallas.tpu as pltpu

S, D, F = 2048, 640, 1728
H, DH, WIN, DIL = 32, 20, 8, 2
NT = D // 128
HALO = 16
LOG2E = math.log2(math.e)
QSCALE = (DH ** -0.5) * LOG2E
NEG = -1e9 * LOG2E
F32 = jnp.float32
BF16 = jnp.bfloat16
U32 = jnp.uint32
I32 = jnp.int32


def _sigmoid(z):
    return 0.5 * jnp.tanh(0.5 * z) + 0.5


def _rows8(v):
    return [v[8 * j:8 * j + 8] for j in range(v.shape[0] // 8)]


def _kernel(x_hbm, wqkv_hbm, wo_hbm, wr_hbm, wg_hbm, wu_hbm, wd_hbm, gw_hbm,
            out_hbm,
            x_v, wqkv_v, wo_v, wr_v, gw_v, wg_v, wu_v, wd_v,
            wqp_v, wkvp_v, wof_v, wop_v, q_s, k_s, v_s, o_s, g_s, xg_s, out_v,
            sem_in, sem_out, *, cfg):
    xt = cfg["x_tiles"]
    pm = cfg["piece"]
    ot = cfg["out_tiles"]
    ka = cfg["ka"]
    npc = S // pm
    nx = len(xt) - 1
    done = set()

    def cp(src, dst, i):
        return pltpu.make_async_copy(src, dst, sem_in.at[i])

    c_wr = cp(wr_hbm, wr_v, 0)
    c_gw = cp(gw_hbm, gw_v, 0)
    c_wqa = cp(wqkv_hbm.at[0:ka, 0:D], wqkv_v.at[0:ka, 0:D], 1)
    c_x = [cp(x_hbm.at[0, xt[i]:xt[i + 1], :], x_v.at[xt[i]:xt[i + 1], :], 2 + i) for i in range(nx)]
    c_wqb = cp(wqkv_hbm.at[ka:D, 0:D], wqkv_v.at[ka:D, 0:D], 3)
    c_wk = cp(wqkv_hbm.at[:, D:2 * D], wqkv_v.at[:, D:2 * D], 1 + nx)
    c_wv = cp(wqkv_hbm.at[:, 2 * D:3 * D], wqkv_v.at[:, 2 * D:3 * D], 1 + nx)
    c_wo = cp(wo_hbm, wo_v, 1 + nx)
    c_wg = cp(wg_hbm, wg_v, 2 + nx)
    c_wu = cp(wu_hbm, wu_v, 2 + nx)
    c_wd = cp(wd_hbm, wd_v, 3 + nx)

    for c in [c_wr, c_gw, c_wqa, c_x[0], c_wqb] + c_x[1:] + [c_wk, c_wv, c_wo, c_wg, c_wu, c_wd]:
        c.start()

    def wait(c):
        c.wait()
        done.add(id(c))

    def need_x(a, b):
        assert all(id(c_x[i]) in done for i in range(nx) if xt[i] < b and xt[i + 1] > a), (a, b)

    for t in range(NT):
        k_s[t, 0:HALO, :] = jnp.zeros((HALO, 128), F32)

    wait(c_wr)
    wait(c_gw)
    wr = wr_v[...].reshape(1, D).astype(F32)
    gw = gw_v[...].reshape(1, D).astype(F32)
    vi = pltpu.bitcast(jnp.broadcast_to(wr[:, 0:128], (8, 128)), I32)
    vz = jnp.maximum(jnp.minimum(vi, 0), 0)
    mfalse = vz != 0
    zi = jnp.max(vz)

    def gated_weights(w_ref, col, gates, k0=0, k1=D):
        gates = [pltpu.bitcast(g, U32) for g in gates]
        lo, hi = k0 // 2, k1 // 2
        parts = [jnp.where(mfalse, g, w_ref[lo + 8 * j:lo + 8 * j + 8, col:col + 128])
                 for j, g in enumerate(gates)]
        if lo + 8 * len(gates) < hi:
            parts.append(w_ref[lo + 8 * len(gates):hi, col:col + 128])
        w = parts[0] if len(parts) == 1 else jnp.concatenate(parts, axis=0)
        return pltpu.bitcast(w, BF16)

    def perm_task(part, r0, prb):
        assert id([c_wqa if r0 < ka else c_wqb, c_wk, c_wv][part]) in done
        lane = jax.lax.broadcasted_iota(I32, (prb // 2, 128), 1)
        lm5 = lane % 5
        src = [pltpu.bitcast(
            wqkv_v[r0:r0 + prb, part * D + t * 128: part * D + (t + 1) * 128], U32)
            for t in range(NT)]
        gates = []
        for t in range(NT):
            bl = src[0]
            for s in range(1, NT):
                bl = jnp.where(lm5 == (t - 3 * s) % 5, src[s], bl)
            pat = ((lane & 31) * DH + 5 * (lane >> 5) + t) & 127
            g = jnp.take_along_axis(bl, pat, axis=1, mode="promise_in_bounds")
            if part == 0:
                wqp_v[r0 // 2:(r0 + prb) // 2, t * 128:(t + 1) * 128] = g
            else:
                c0 = (part - 1) * D + t * 128
                wkvp_v[r0 // 2:(r0 + prb) // 2, c0:c0 + 128] = g
            gates += _rows8(g)
        done.update(("perm", part, r) for r in range(r0, r0 + prb, 16))
        return gates

    def wo_task(j, t):
        assert id(c_wo) in done
        if t == 0:
            wof_v[j, 0:D, :] = wo_v[:, j * 128:(j + 1) * 128].astype(F32)
        gates = []
        for c in range(4):
            rows = wof_v[j, pl.ds(5 * c + t, H, stride=DH), :]
            pk = pltpu.bitcast(rows.astype(BF16), U32)
            r0 = (t * 128 + c * H) // 2
            wop_v[r0:r0 + H // 2, j * 128:(j + 1) * 128] = pk
            gates += _rows8(pk)
        done.add(("wop", j, t))
        return gates

    sub = jax.lax.broadcasted_iota(I32, (8, 128), 0)
    st = dict(best_v=jnp.full((8, 128), -jnp.inf, F32), best_i=jnp.zeros((8, 128), I32))
    rvals = {}

    def rg_task(r0):
        need_x(r0, r0 + 16)
        xf16 = x_v[r0:r0 + 16, :].astype(F32)
        gates = []
        for hh in range(2):
            xf = xf16[hh * 8:(hh + 1) * 8]
            xs = [xf[:, t * 128:(t + 1) * 128] for t in range(NT)]
            pr = xs[0] * wr[:, 0:128]
            pg = xs[0] * gw[:, 0:128]
            for t in range(1, NT):
                pr = pr + xs[t] * wr[:, t * 128:(t + 1) * 128]
                pg = pg + xs[t] * gw[:, t * 128:(t + 1) * 128]
            rr = r0 + hh * 8
            rvals[rr] = jnp.broadcast_to(jnp.sum(pr, axis=1, keepdims=True), (8, 128))
            gates.append(rvals[rr])
            g = jnp.broadcast_to(_sigmoid(jnp.sum(pg, axis=1, keepdims=True)), (8, 128))
            g_s[rr:rr + 8, :] = g
            omg = 1.0 - g
            for t in range(NT):
                xg = omg * xs[t]
                xg_s[t, rr:rr + 8, :] = xg
                gates.append(xg)
        done.add(("rg", r0))
        return gates

    def argmax_task(a, b):
        for rr in range(a, b, 8):
            rv = rvals.pop(rr).astype(BF16).astype(F32)
            upd = rv > st["best_v"]
            st["best_v"] = jnp.where(upd, rv, st["best_v"])
            st["best_i"] = jnp.where(upd, sub + rr, st["best_i"])
        return [st["best_v"], st["best_i"]]

    def sel_task():
        assert not rvals and all(("rg", r) in done for r in range(0, S, 16))
        best_v, best_i = st["best_v"], st["best_i"]
        top_v = jnp.max(best_v, axis=0, keepdims=True)
        cand = jnp.where(best_v == top_v, best_i, S)
        top_i = jnp.min(cand, axis=0, keepdims=True)
        idx = jnp.clip(jnp.min(top_i), 0, S - 1)
        base = pl.multiple_of((idx >> 4) << 4, 16)
        xblk = x_v[pl.ds(base, 16), :].astype(F32)
        rsel = jax.lax.broadcasted_iota(I32, (16, D), 0) == (idx - base)
        x_sel = jnp.sum(jnp.where(rsel, xblk, 0.0), axis=0, keepdims=True)
        st.update(top_v=top_v, top_i=top_i, base=base, x_sel=x_sel)
        return []

    accs = [jnp.zeros((8, 128), F32) for _ in range(NT)]
    hvals = {}

    def gu_task(k0):
        assert id(c_wg) in done and id(c_wu) in done
        x_sel = st["x_sel"]
        gt = jnp.sum(wg_v[k0:k0 + 16, :].astype(F32) * x_sel, axis=1, keepdims=True)
        ut = jnp.sum(wu_v[k0:k0 + 16, :].astype(F32) * x_sel, axis=1, keepdims=True)
        hvals[k0] = jnp.broadcast_to(gt * _sigmoid(gt) * ut, (16, 128))
        return _rows8(hvals[k0])

    def dn_task(k0, k1):
        assert id(c_wd) in done
        for k in range(k0, k1, 16):
            hc = hvals.pop(k)
            for t in range(NT):
                p = wd_v[k:k + 16, t * 128:(t + 1) * 128].astype(F32) * hc
                accs[t] = accs[t] + (p[0:8] + p[8:16])
            done.add(("dn", k))
        return list(accs)

    def ffn_fin(done_rows):
        assert all(("dn", k) in done for k in range(0, F, 16))
        assert all((("out", r, t) in done) == (r < done_rows) for r in range(0, S, 16) for t in range(NT))
        gsel = _sigmoid(jnp.sum(st["x_sel"] * gw, axis=1, keepdims=True))
        sc = _sigmoid(st["top_v"]) * (1.0 - gsel)
        y = [jnp.sum(accs[t], axis=0, keepdims=True) * sc for t in range(NT)]
        row16 = jax.lax.broadcasted_iota(I32, (16, 128), 0)
        base = st["base"]
        hit = (row16 + base) == st["top_i"]
        pb = pl.multiple_of(jnp.minimum(base, done_rows - 16), 16)
        hit2 = (row16 + pb) == st["top_i"]
        for t in range(NT):
            xg_s[t, pl.ds(base, 16), :] = xg_s[t, pl.ds(base, 16), :] + jnp.where(hit, y[t], 0.0)
            cur = out_v[pl.ds(pb, 16), t * 128:(t + 1) * 128].astype(F32)
            out_v[pl.ds(pb, 16), t * 128:(t + 1) * 128] = (cur + jnp.where(hit2, y[t], 0.0)).astype(BF16)
        done.add("fin")
        return []

    def rows(ref, t, off):
        return ref[t, pl.ds(off, 8, stride=2), :]

    staged = {}

    def attn_a(r0, gate=False):
        if r0 in staged:
            return []
        assert all((kind, r0 // 16 * 16, t) in done for kind in "qk" for t in range(NT))
        qs = [rows(q_s, t, r0) for t in range(NT)]
        ps = []
        for w in range(WIN):
            off = HALO + r0 - DIL * w
            acc = qs[0] * rows(k_s, 0, off)
            for t in range(1, NT):
                acc = acc + qs[t] * rows(k_s, t, off)
            ps.append(acc)
        staged[r0] = [p + pltpu.roll(p, 64, 1) for p in ps]
        return list(staged[r0]) if gate else []

    def attn_b(r0):
        attn_a(r0)
        assert all(("v", r0 // 16 * 16, t) in done for t in range(NT)) and ("rg", r0 // 16 * 16) in done
        logits = [p + pltpu.roll(p, 32, 1) for p in staged[r0]]
        staged[r0] = None
        for w in range(WIN):
            if r0 < DIL * w:
                logits[w] = jnp.where(2 * sub + r0 >= DIL * w, logits[w], NEG)
        m = logits[0]
        for w in range(1, WIN):
            m = jnp.maximum(m, logits[w])
        es = [jnp.exp2(l - m) for l in logits]
        den = es[0]
        for w in range(1, WIN):
            den = den + es[w]
        rc = pl.reciprocal(den, approx=True)
        inv = rc * (2.0 - den * rc) * g_s[pl.ds(r0, 8, stride=2), :]
        outs = []
        for t in range(NT):
            acc = es[0] * rows(v_s, t, HALO + r0)
            for w in range(1, WIN):
                acc = acc + es[w] * rows(v_s, t, HALO + r0 - DIL * w)
            outs.append(acc * inv)
            o_s[t, pl.ds(r0, 8, stride=2), :] = outs[-1]
        done.add(("o", r0))
        return outs

    outs_dma = []

    def send_task(a, b, c0, c1):
        assert "fin" in done
        assert all(("out", r, t) in done for r in range(a, b, 16) for t in range(c0 // 128, c1 // 128))
        c = pltpu.make_async_copy(out_v.at[a:b, c0:c1], out_hbm.at[0, a:b, c0:c1], sem_out.at[0])
        c.start()
        outs_dma.append(c)
        done.update(("sent", r, t) for r in range(a, b, 16) for t in range(c0 // 128, c1 // 128))
        return []

    def out_fence():
        r = pl.multiple_of(S + zi * 16, 16)
        out_v[pl.ds(r, 16), 0:128] = jnp.zeros((16, 128), BF16)
        return [out_v[pl.ds(r, 16), 0:128]]

    olag = cfg["out_lag"]
    am = cfg["qa_rows"]
    ops = [("qa", a, a + am) for a in range(0, xt[2], am)]
    ops += [("qb", a, a + pm) for a in range(0, xt[2], pm)]
    ops += [("q", a, a + pm) for a in range(xt[2], S, pm)]
    for i in range(npc + olag):
        if i < npc:
            ops.append(("kv", i * pm, (i + 1) * pm))
        if i >= olag:
            p = i - olag
            cuts = [p * pm + c for c in cfg["last_cuts"]] if p == npc - 1 else [p * pm, (p + 1) * pm]
            ops += [("wo", a, b) for a, b in zip(cuts[:-1], cuts[1:])]
    ktiles = {"qa": ka // 128, "qb": NT - ka // 128}
    slots, T = [], [0]
    for kind, a, b in ops:
        for t in range(2 * NT if kind == "kv" else NT):
            slots.append((kind, a, b, t))
            T.append(T[-1] + (b - a) * ktiles.get(kind, NT) // 4)
    ns = len(slots)
    first, last = {}, {}
    for n_, (kind, a, b, t) in enumerate(slots):
        for r in range(a, b, 16):
            first.setdefault((kind, r), n_)
            last[(kind, r)] = n_

    def at(time):
        return min(bisect.bisect_left(T, time), ns)

    tasks = [[] for _ in range(ns + 1)]
    waits = {}

    def spread(fns, t0, t1):
        for n_, fn in enumerate(fns):
            tasks[at(t0 + (t1 - t0) * (n_ + 1) // len(fns))].append(fn)

    t2 = T[first[("kv", 0)]]
    fw1, fw2 = at(t2 + cfg["gu_wait"]), at(t2 + cfg["dn_wait"])
    bars = [first[("qa" if i < 2 else "q", xt[i])] for i in range(nx)] + [fw1]
    for i in range(nx):
        waits[bars[i]] = [c_x[i]]
    waits[bars[1]] += [c_wqb]
    waits[bars[nx - 1]] += [c_wk, c_wv, c_wo]
    waits[fw1] = [c_wg, c_wu]
    waits[fw2] = [c_wd]
    blk = cfg["blackout"]
    rcuts = cfg["rg_cuts"]
    for i in range(1, nx):
        t0, t1 = T[bars[i]] + blk, T[bars[i + 1]]
        if i == 1:
            t0 = T[first[("qb", 0)]]
        if i == nx - 1:
            t0, t1 = t2 + cfg["rg_head"], t2 + cfg["rg_tail"]
        spread([functools.partial(rg_task, r0) for r0 in range(rcuts[i - 1], rcuts[i], 16)], t0, t1)
        if i < nx - 1:
            na = cfg["argmax_n"]
            cuts = [rcuts[i - 1] + (rcuts[i] - rcuts[i - 1]) // 8 * j // na * 8 for j in range(na + 1)]
            spread([functools.partial(argmax_task, cuts[j], cuts[j + 1]) for j in range(na)],
                   T[bars[i + 1]] + 160, T[bars[i + 1]] + 160 + 320 * na)
    spread([functools.partial(perm_task, 0, r0, 32) for r0 in range(ka, D, 32)],
           T[bars[1]] + cfg["permb_off"], T[first[("qb", 0)] - 1])
    prb = cfg["perm_rb"]
    p0, p1 = T[bars[nx - 1]] + blk, t2 + 640
    mid = min((p0 + p1) // 2, t2 - 160)
    spread([functools.partial(perm_task, 1, r0, prb) for r0 in range(0, D, prb)], p0, mid)
    spread([functools.partial(perm_task, 2, r0, prb) for r0 in range(0, D, prb)], mid, p1)
    spread([functools.partial(wo_task, j, t) for j in range(NT) for t in range(NT)],
           t2 + cfg["wo_0"], t2 + cfg["wo_1"])
    tasks[at(T[fw1] + cfg["sel_off"])] += [functools.partial(argmax_task, rcuts[-2], rcuts[-1]), sel_task]
    spread([functools.partial(gu_task, k0) for k0 in range(0, F, 16)], T[fw1] + cfg["gu_off"], T[fw2])
    dg = cfg["dn_group"] * 16
    spread([functools.partial(dn_task, k0, min(k0 + dg, F)) for k0 in range(0, F, dg)],
           T[fw2] + 160, t2 + cfg["ffn_end"])
    tasks[last[("wo", ot[1] - 16)] + 1].append(functools.partial(ffn_fin, ot[1]))
    aoff, ablk = cfg["attn_off"], cfg["attn_blk"]
    a0 = T[last[("kv", 0)] + 1] + aoff
    a1 = T[first[("wo", S - 16)]]
    nat = S // 8
    span = a1 - a0 - 2 * ablk
    prev = 0
    for j in range(nat):
        r0 = j // 2 * 16
        tm = a0 + span * j // (nat - 1)
        for w in (fw1, fw2):
            if tm > T[w]:
                tm += ablk
        lo = T[last[("kv", r0)] + 1] + aoff + (j % (pm // 8)) * cfg["attn_gap"]
        s = min(max(at(tm), at(lo), prev), first[("wo", r0)])
        while any(T[w] < T[s] < T[w] + ablk for w in (fw1, fw2)):
            s += 1
        prev = s
        for c in range(j + 1, min(j + cfg["a_ahead"] + 1, nat)):
            if T[last[("kv", c // 2 * 16)] - NT + 1] + aoff <= T[s]:
                tasks[s].append(functools.partial(attn_a, c // 2 * 16 + c % 2, True))
        tasks[s].append(functools.partial(attn_b, r0 + j % 2))
    cs = cfg["split_last"]
    for n_, (kind, a, b, t) in enumerate(slots):
        if kind != "wo":
            continue
        if b == S:
            if t == cs - 1:
                tasks[n_ + 1].append(functools.partial(send_task, a, b, 0, cs * 128))
            if t == NT - 1:
                tasks[n_ + 1].append(functools.partial(send_task, a, b, cs * 128, D))
        elif t == NT - 1:
            if b in ot:
                tasks[n_ + 1].append(functools.partial(send_task, ot[ot.index(b) - 1], b, 0, D))
            s = at(T[n_ + 1] + cfg["ofence_off"])
            if s < ns:
                tasks[n_ + 1].append(("fence", s))

    wait(c_wqa)
    perm_task(0, 0, ka)

    xl = {}

    def x_rows(a, b):
        need_x(a, b)
        for r in range(a, b, 64):
            if r not in xl:
                xl[r] = x_v[r:r + 64, :]
        parts = [xl[r] for r in range(a, b, 64)]
        return parts[0] if len(parts) == 1 else jnp.concatenate(parts, axis=0)

    def need_perm(part, k0, k1):
        assert all(("perm", part, r) in done for r in range(k0, k1, 16)), (part, k0, k1)

    carry = []
    later = {}
    qpart = {}
    for s in range(ns + 1):
        gates = carry + later.pop(s, [])
        for fn in tasks[s]:
            if isinstance(fn, tuple):
                later.setdefault(fn[1], []).extend(out_fence())
            else:
                gates += fn()
        if s in waits:
            for c in waits[s]:
                wait(c)
            gates = []
        if s == ns:
            break
        kind, a, b, t = slots[s]
        cap = ktiles.get(kind, NT) * 8
        gates, carry = gates[:cap], gates[cap:]
        mark = None
        if kind == "qa":
            need_perm(0, 0, ka)
            r = jnp.dot(x_rows(a, b)[:, 0:ka], gated_weights(wqp_v, t * 128, gates, 0, ka),
                        preferred_element_type=F32)
            for r0 in range(a, b, 64):
                qpart[(r0, t)] = r[r0 - a:r0 - a + 64]
        elif kind == "qb":
            need_perm(0, ka, D)
            q = jnp.dot(x_rows(a, b)[:, ka:D], gated_weights(wqp_v, t * 128, gates, ka, D),
                        preferred_element_type=F32)
            for r0 in range(a, b, 64):
                q_s[t, r0:r0 + 64, :] = (q[r0 - a:r0 - a + 64] + qpart.pop((r0, t))) * QSCALE
            mark = ("q", t)
        elif kind == "q":
            q = jnp.dot(x_rows(a, b), gated_weights(wqp_v, t * 128, gates), preferred_element_type=F32)
            q_s[t, a:b, :] = q * QSCALE
            mark = ("q", t)
        elif kind == "kv":
            need_perm(1 + t // NT, 0, D)
            r = jnp.dot(x_rows(a, b), gated_weights(wkvp_v, t * 128, gates), preferred_element_type=F32)
            if t < NT:
                k_s[t, HALO + a:HALO + b, :] = r
            else:
                v_s[t - NT, HALO + a:HALO + b, :] = r
                if a == 0:
                    v_s[t - NT, 0:HALO, :] = jnp.broadcast_to(r[0:1], (HALO, 128))
            mark = ("kv"[t // NT], t % NT)
        else:
            assert all(("wop", t, n_) in done for n_ in range(NT))
            if t == 0:
                assert all(("o", r + par) in done for r in range(a, b, 16) for par in range(2))
                ol = jnp.concatenate([o_s[n_, a:b, :] for n_ in range(NT)], axis=1).astype(BF16)
            att = jnp.dot(ol, gated_weights(wop_v, t * 128, gates), preferred_element_type=F32)
            out_v[a:b, t * 128:(t + 1) * 128] = (att + xg_s[t, a:b, :]).astype(BF16)
            mark = ("out", t)
        if mark:
            done.update((mark[0], r, mark[1]) for r in range(a, b, 16))
    assert all(("sent", r, t) in done for r in range(0, S, 16) for t in range(NT))
    for c in outs_dma:
        c.wait()


_CFG = dict(
    x_tiles=(0, 256, 512, 1536, 2048), ka=384, qa_rows=64, piece=128,
    rg_cuts=(0, 128, 1536, 2048),
    out_tiles=(0, 1152, 1408, 1664, 1792, 1920, 1984, 2048),
    last_cuts=(0, 64, 128), split_last=4,
    perm_rb=32, permb_off=300, blackout=320, rg_head=-960, rg_tail=2560,
    wo_0=640, wo_1=4800, sel_off=480, argmax_n=4,
    out_lag=3, attn_off=480, attn_gap=80, attn_blk=640, a_ahead=2, ofence_off=640,
    gu_wait=5760, gu_off=960, dn_wait=16000, ffn_end=25600, dn_group=3,
)


def _build(cfg):
    hbm = pl.BlockSpec(memory_space=pltpu.HBM)
    n_in = 4 + len(cfg["x_tiles"]) - 1
    return pl.pallas_call(
        functools.partial(_kernel, cfg=cfg),
        out_shape=jax.ShapeDtypeStruct((1, S, D), BF16),
        in_specs=[hbm] * 8,
        out_specs=hbm,
        scratch_shapes=[
            pltpu.VMEM((S, D), BF16),
            pltpu.VMEM((D, 3 * D), BF16),
            pltpu.VMEM((D, D), BF16),
            pltpu.VMEM((D,), BF16),
            pltpu.VMEM((D,), BF16),
            pltpu.VMEM((F, D), BF16),
            pltpu.VMEM((F, D), BF16),
            pltpu.VMEM((F, D), BF16),
            pltpu.VMEM((D // 2, D), U32),
            pltpu.VMEM((D // 2, 2 * D), U32),
            pltpu.VMEM((NT, D + 40, 128), F32),
            pltpu.VMEM((D // 2, D), U32),
            pltpu.VMEM((NT, S + 8, 128), F32),
            pltpu.VMEM((NT, S + HALO + 8, 128), F32),
            pltpu.VMEM((NT, S + HALO + 8, 128), F32),
            pltpu.VMEM((NT, S + 8, 128), F32),
            pltpu.VMEM((S + 8, 128), F32),
            pltpu.VMEM((NT, S, 128), F32),
            pltpu.VMEM((S + 16, D), BF16),
            pltpu.SemaphoreType.DMA((n_in,)),
            pltpu.SemaphoreType.DMA((1,)),
        ],
        compiler_params=pltpu.CompilerParams(vmem_limit_bytes=100 * 1024 * 1024),
        name="gated_mix_kernel",
    )


@jax.jit
def pallas_gated_mix__sliding_local_dilated__moe_arch_mod__prompt_kernel(
    A_x: jax.Array,
    A_wqkv: jax.Array,
    A_wo: jax.Array,
    B_x: jax.Array,
    B_w_r: jax.Array,
    B_w_gate: jax.Array,
    B_w_up: jax.Array,
    B_w_down: jax.Array,
    gate_w: jax.Array,
):
    del B_x
    return _build(_CFG)(A_x, A_wqkv, A_wo, B_w_r, B_w_gate.T, B_w_up.T, B_w_down, gate_w)
```
